```python
import os as _os
_os.environ.setdefault("JAX_PLATFORMS", "cpu")
import jax
import jax.numpy as jnp

def _softmax(x, axis=-1):
    return jax.nn.softmax(x, axis=axis)
def _gelu(x):
    return jax.nn.gelu(x, approximate=True)
def _silu(x):
    return jax.nn.silu(x)
def _sigmoid(x):
    return jax.nn.sigmoid(x)
def _layernorm(x, axis=-1, eps=1e-5):
    m = jnp.mean(x, axis=axis, keepdims=True)
    v = jnp.var(x, axis=axis, keepdims=True)
    return (x - m) / jnp.sqrt(v + eps)
def _scatter_add(tgt, idx, src, axis=0):
    return tgt.at[idx].add(src)
def _segment_sum(src, seg, n):
    return jax.ops.segment_sum(src, seg, n)
class _Rng:
    def __init__(self, key):
        self._k = key
    def _next(self):
        self._k, sub = jax.random.split(self._k)
        return sub
    def normal(self, shape):
        return jax.random.normal(self._next(), shape, dtype=jnp.bfloat16)
    def randint(self, lo, hi, shape):
        return jax.random.randint(self._next(), shape, lo, hi, dtype=jnp.int32)
    def uniform(self, shape, lo=0.0, hi=1.0):
        return jax.random.uniform(self._next(), shape, jnp.bfloat16, lo, hi)
    def permutation(self, n):
        return jax.random.permutation(self._next(), n)


kernel_name = 'standalone__mha_softmax__near_ridge'

def setup_inputs():
    _rng = _Rng(jax.random.key(int.from_bytes(__import__("os").urandom(4), "little")))
    _w = (lambda a: (lambda t: t.astype(jnp.bfloat16) if jnp.issubdtype(t.dtype, jnp.floating) else t)(jnp.asarray(a)))
    B, H, Sq, Sk, D = 8, 32, 304, 2048, 128
    return {
        "q": _w((lambda *s: _rng.normal(s) * 0.4)(B, H, Sq, D)),
        "k": _w((lambda *s: _rng.normal(s) * 0.4)(B, H, Sk, D)),
        "v": _w((lambda *s: _rng.normal(s) * 0.05)(B, H, Sk, D)),
    }

def reference(q, k, v):
    scale = q.shape[-1] ** -0.5
    scores = jnp.einsum("bhqd,bhkd->bhqk", q, k) * scale
    p = _softmax(scores, axis=-1)
    return jnp.einsum("bhqk,bhkd->bhqd", p, v)
```

```python
import jax
import jax.numpy as jnp
import numpy as np
from jax import lax
import jax.experimental.pallas as pl
import jax.experimental.pallas.tpu as pltpu

_LOG2E = 1.4426950408889634
_NT = (((1,), (1,)), ((), ()))
_NN = (((1,), (0,)), ((), ()))

_U = 8
_CK = 512
_LANES = 128


def _ld(ref):
    return pltpu.bitcast(ref.bitcast(jnp.uint32)[...], jnp.bfloat16)


def _stage(q_ref, k_ref, v_ref, o_ref, s_in, m_in, r_prev, true_mask, scale):
    do_qk = q_ref is not None
    do_pv = v_ref is not None
    sk = (k_ref if do_qk else v_ref).shape[0]
    nt = _CK // _LANES
    s_out = []
    m_run = l_run = acc = None
    if do_qk:
        qh = (_ld(q_ref).astype(jnp.float32) * scale).astype(jnp.bfloat16)
    for j in range(sk // _CK):
        keys = pl.ds(j * _CK, _CK)
        if do_qk:
            s = lax.dot_general(qh, _ld(k_ref.at[keys, :]), _NT,
                                preferred_element_type=jnp.float32)
            tiles = [s[:, t * _LANES:(t + 1) * _LANES] for t in range(nt)]
            s_out.append((s, tiles))
            for st in tiles:
                m_run = st if m_run is None else jnp.maximum(m_run, st)
        if do_pv:
            m_j = m_in if r_prev is None else jnp.where(true_mask, m_in, r_prev)
            p = [jnp.exp2(s_in(j, t) - m_j) for t in range(nt)]
            part = (p[0] + p[1]) + (p[2] + p[3])
            l_run = part if l_run is None else l_run + part
            p[-1] = jnp.minimum(p[-1], l_run)
            pb = jnp.concatenate(p, axis=1).astype(jnp.bfloat16)
            r_prev = lax.dot_general(pb, _ld(v_ref.at[keys, :]), _NN,
                                     preferred_element_type=jnp.float32)
            acc = r_prev if acc is None else acc + r_prev
    m_out = None
    if do_qk:
        m_out = jnp.broadcast_to(jnp.max(m_run, axis=-1, keepdims=True), m_run.shape)
    if do_pv:
        l = jnp.sum(l_run, axis=-1, keepdims=True)
        r0 = pl.reciprocal(l, approx=True)
        inv = r0 * (2.0 - l * r0)
        o_ref[...] = (acc * inv).astype(o_ref.dtype)
    return s_out, m_out, r_prev


def _make_kernel(bh, sq, sk, d):
    n_it = bh // _U
    scale = np.float32(d ** -0.5 * _LOG2E)

    def kernel(q_hbm, k_hbm, v_hbm, o_hbm, qb, kb, vb, ob, q0b, k0b, s_buf, m_buf,
               qsem, ksem, vsem, osem, psem):
        def kq_copies(g, u):
            h = g * _U + u + 1
            if u == _U - 1:
                h = jnp.minimum(h, bh - 1)
            return [pltpu.make_async_copy(k_hbm.at[h], kb.at[u], ksem.at[u]),
                    pltpu.make_async_copy(q_hbm.at[h], qb.at[u], qsem.at[u])]

        def v_copy(g, u):
            return pltpu.make_async_copy(v_hbm.at[g * _U + u], vb.at[u], vsem.at[u])

        def o_copy(g, oslot):
            return pltpu.make_async_copy(
                ob.at[oslot], o_hbm.at[pl.ds(g * _U, _U)], osem.at[oslot])

        def start_in(g, u):
            for cp in kq_copies(g, u):
                cp.start()
            v_copy(g, u).start()

        def wait_in(g, u):
            for cp in kq_copies(g, u):
                cp.wait()
            v_copy(g, u).wait()

        def store_scores(s_out, m_out):
            for j, (s, _) in enumerate(s_out):
                s_buf[:, pl.ds(j * _CK, _CK)] = s
            m_buf[...] = m_out

        first = [pltpu.make_async_copy(q_hbm.at[0], q0b, psem.at[0]),
                 pltpu.make_async_copy(k_hbm.at[0], k0b, psem.at[1])]
        for cp in first:
            cp.start()
        start_in(0, 0)
        for cp in first:
            cp.wait()
        for u in range(1, _U):
            start_in(0, u)
        s_out, m_out, _ = _stage(q0b, k0b, None, None, None, None, None, None, scale)
        store_scores(s_out, m_out)

        def body(g, carry):
            oslot = lax.rem(g, 2)

            @pl.when(g >= 2)
            def _():
                o_copy(g - 2, oslot).wait()

            @pl.when(g >= 1)
            def _():
                o_copy(g - 1, 1 - oslot).start()

            bits = lax.bitcast_convert_type(
                q0b.at[pl.ds(0, 16), :].bitcast(jnp.uint32)[...], jnp.int32)
            true_mask = (bits | 1) != 0
            true_mask = jnp.broadcast_to(
                true_mask.reshape(1, 8, _LANES), (sq // 8, 8, _LANES)).reshape(sq, _LANES)

            s_in = lambda j, t: s_buf[:, pl.ds(j * _CK + t * _LANES, _LANES)]
            m_in = m_buf[...]
            r_prev = None
            for u in range(_U):
                wait_in(g, u)
                s_out, m_out, r_prev = _stage(
                    qb.at[u], kb.at[u], vb.at[u], ob.at[oslot, u],
                    s_in, m_in, r_prev, true_mask, scale)
                if u == _U - 1:
                    store_scores(s_out, m_out)
                else:
                    s_in = lambda j, t, s_out=s_out: s_out[j][1][t]
                    m_in = m_out

                @pl.when(g + 1 < n_it)
                def _():
                    start_in(g + 1, u)

            return carry

        lax.fori_loop(0, n_it, body, 0)
        o_copy(n_it - 2, (n_it - 2) % 2).wait()
        o_copy(n_it - 1, (n_it - 1) % 2).start()
        o_copy(n_it - 1, (n_it - 1) % 2).wait()

    return kernel


@jax.jit
def pallas_standalone__mha_softmax__near_ridge_kernel(
    q: jax.Array,
    k: jax.Array,
    v: jax.Array,
):
    b, h, sq, d = q.shape
    sk = k.shape[2]
    bh = b * h
    assert d == _LANES and sk % _CK == 0 and sq % 16 == 0 and bh % _U == 0 and bh >= 2 * _U

    dt = q.dtype
    out = pl.pallas_call(
        _make_kernel(bh, sq, sk, d),
        in_specs=[pl.BlockSpec(memory_space=pl.ANY)] * 3,
        out_specs=pl.BlockSpec(memory_space=pl.ANY),
        out_shape=jax.ShapeDtypeStruct((bh, sq, d), dt),
        scratch_shapes=[
            pltpu.VMEM((_U, sq, d), dt),
            pltpu.VMEM((_U, sk, d), dt),
            pltpu.VMEM((_U, sk, d), dt),
            pltpu.VMEM((2, _U, sq, d), dt),
            pltpu.VMEM((sq, d), dt),
            pltpu.VMEM((sk, d), dt),
            pltpu.VMEM((sq, sk), jnp.float32),
            pltpu.VMEM((sq, _LANES), jnp.float32),
            pltpu.SemaphoreType.DMA((_U,)),
            pltpu.SemaphoreType.DMA((_U,)),
            pltpu.SemaphoreType.DMA((_U,)),
            pltpu.SemaphoreType.DMA((2,)),
            pltpu.SemaphoreType.DMA((2,)),
        ],
        compiler_params=pltpu.CompilerParams(
            vmem_limit_bytes=100 * 1024 * 1024,
            flags={"XLA_TPU_RESCHEDULE_DMA_DONES": True},
        ),
    )(q.reshape(bh, sq, d), k.reshape(bh, sk, d), v.reshape(bh, sk, d))
    return out.reshape(b, h, sq, d)
```

```python
import jax
import jax.numpy as jnp
import numpy as np
from jax import lax
import jax.experimental.pallas as pl
import jax.experimental.pallas.tpu as pltpu

_LOG2E = 1.4426950408889634
_NT = (((1,), (1,)), ((), ()))
_NN = (((1,), (0,)), ((), ()))

_LANES = 128
_CK = 512
_U = 15
_NB = 5
_OG = 5
_NOS = 2 * (_U // _OG)


def _ld(ref):
    return pltpu.bitcast(ref.bitcast(jnp.uint32)[...], jnp.bfloat16)


def _stage(q_ref, k_ref, v_ref, o_ref, s_in, m_in, r_prev, true_mask, scale):
    do_qk = q_ref is not None
    do_pv = v_ref is not None
    pace = do_qk and do_pv
    sk = (k_ref if do_qk else v_ref).shape[0]
    nt = _CK // _LANES
    s_out = []
    m_run = l_run = acc = None
    if do_qk:
        qh = (_ld(q_ref).astype(jnp.float32) * scale).astype(jnp.bfloat16)
    for j in range(sk // _CK):
        keys = pl.ds(j * _CK, _CK)
        if do_qk:
            s = lax.dot_general(qh, _ld(k_ref.at[keys, :]), _NT,
                                preferred_element_type=jnp.float32)
            tiles = [s[:, t * _LANES:(t + 1) * _LANES] for t in range(nt)]
            s_out.append((s, tiles))
            mx = jnp.maximum(jnp.maximum(tiles[0], tiles[1]),
                             jnp.maximum(tiles[2], tiles[3]))
            m_run = mx if m_run is None else jnp.maximum(m_run, mx)
        if do_pv:
            m_j = m_in
            if pace and r_prev is not None:
                m_j = jnp.where(true_mask, m_in, r_prev)
            p = [jnp.exp2(s_in(j, t) - m_j) for t in range(nt)]
            part = (p[0] + p[1]) + (p[2] + p[3])
            l_run = part if l_run is None else l_run + part
            if pace:
                for t in (1, 3):
                    p[t] = jnp.minimum(p[t], l_run)
            pb = jnp.concatenate(p, axis=1).astype(jnp.bfloat16)
            r_prev = lax.dot_general(pb, _ld(v_ref.at[keys, :]), _NN,
                                     preferred_element_type=jnp.float32)
            acc = r_prev if acc is None else acc + r_prev
    m_out = None
    if do_qk:
        m_out = jnp.broadcast_to(jnp.max(m_run, axis=-1, keepdims=True), m_run.shape)
    if do_pv:
        l = jnp.sum(l_run, axis=-1, keepdims=True)
        r0 = pl.reciprocal(l, approx=True)
        inv = r0 * (2.0 - l * r0)
        o_ref[...] = (acc * inv).astype(o_ref.dtype)
    return s_out, m_out, r_prev


def _make_kernel(bh, sq, sk, d):
    n_it = (bh - 1) // _U
    n_og = _U // _OG
    n_grp = n_it * n_og
    scale = np.float32(d ** -0.5 * _LOG2E)

    def kernel(q_hbm, k_hbm, v_hbm, o_hbm,
               qb, kb, vb, ob, q0b, k0b, vlb, olb, s_buf, m_buf,
               qsem, ksem, vsem, osem, psem, lsem):
        def in_copies(g, u):
            h, slot = g * _U + u, u % _NB
            return [pltpu.make_async_copy(k_hbm.at[h + 1], kb.at[slot], ksem.at[slot]),
                    pltpu.make_async_copy(q_hbm.at[h + 1], qb.at[slot], qsem.at[slot]),
                    pltpu.make_async_copy(v_hbm.at[h], vb.at[slot], vsem.at[slot])]

        def start_in(g, u):
            for cp in in_copies(g, u):
                cp.start()

        def wait_in(g, u):
            for cp in in_copies(g, u):
                cp.wait()

        def o_copy(n, slot):
            return pltpu.make_async_copy(
                ob.at[slot], o_hbm.at[pl.ds(n * _OG, _OG)], osem.at[slot])

        def store_scores(s_out, m_out):
            for j, (s, _) in enumerate(s_out):
                s_buf[:, pl.ds(j * _CK, _CK)] = s
            m_buf[...] = m_out

        def load_scores(j, t):
            return s_buf[:, pl.ds(j * _CK + t * _LANES, _LANES)]

        def make_true_mask():
            bits = lax.bitcast_convert_type(
                q0b.at[pl.ds(0, 16), :].bitcast(jnp.uint32)[...], jnp.int32)
            mask = (bits | 1) != 0
            return jnp.broadcast_to(mask.reshape(1, 8, _LANES),
                                    (sq // 8, 8, _LANES)).reshape(sq, _LANES)

        v_last = pltpu.make_async_copy(v_hbm.at[bh - 1], vlb, lsem.at[0])
        o_last = pltpu.make_async_copy(olb, o_hbm.at[bh - 1], lsem.at[1])

        first = [pltpu.make_async_copy(q_hbm.at[0], q0b, psem.at[0]),
                 pltpu.make_async_copy(k_hbm.at[0], k0b, psem.at[1])]
        for cp in first:
            cp.start()
        start_in(0, 0)
        for cp in first:
            cp.wait()
        for u in range(1, _NB):
            start_in(0, u)
        s_out, m_out, _ = _stage(q0b, k0b, None, None, None, None, None, None, scale)
        store_scores(s_out, m_out)

        def body(g, carry):
            true_mask = make_true_mask()
            s_in, m_in, r_prev = load_scores, m_buf[...], None
            for u in range(_U):
                n = g * n_og + u // _OG
                oslot = lax.rem(n, _NOS)
                if u % _OG == 0:
                    @pl.when(n >= _NOS)
                    def _():
                        o_copy(n - _NOS, oslot).wait()

                    @pl.when(n >= 1)
                    def _():
                        o_copy(n - 1, lax.rem(n + _NOS - 1, _NOS)).start()

                wait_in(g, u)
                slot = u % _NB
                s_out, m_out, r_prev = _stage(
                    qb.at[slot], kb.at[slot], vb.at[slot], ob.at[oslot, u % _OG],
                    s_in, m_in, r_prev, true_mask, scale)
                if u == _U - 1:
                    store_scores(s_out, m_out)
                else:
                    s_in = lambda j, t, s_out=s_out: s_out[j][1][t]
                    m_in = m_out

                if u + _NB < _U:
                    start_in(g, u + _NB)
                else:
                    @pl.when(g + 1 < n_it)
                    def _():
                        start_in(g + 1, u + _NB - _U)

                    if u + _NB == _U:
                        @pl.when(g + 1 == n_it)
                        def _():
                            v_last.start()
            return carry

        lax.fori_loop(0, n_it, body, 0)

        o_copy(n_grp - 1, (n_grp - 1) % _NOS).start()
        v_last.wait()
        _stage(None, None, vlb, olb, load_scores, m_buf[...], None, None, scale)
        o_last.start()
        for n in range(max(n_grp - _NOS, 0), n_grp):
            o_copy(n, n % _NOS).wait()
        o_last.wait()

    return kernel


@jax.jit
def pallas_standalone__mha_softmax__near_ridge_kernel(
    q: jax.Array,
    k: jax.Array,
    v: jax.Array,
):
    b, h, sq, d = q.shape
    sk = k.shape[2]
    bh = b * h
    assert d == _LANES and sk % _CK == 0 and sq % 16 == 0
    assert bh > _U and (bh - 1) % _U == 0

    dt = q.dtype
    out = pl.pallas_call(
        _make_kernel(bh, sq, sk, d),
        in_specs=[pl.BlockSpec(memory_space=pl.ANY)] * 3,
        out_specs=pl.BlockSpec(memory_space=pl.ANY),
        out_shape=jax.ShapeDtypeStruct((bh, sq, d), dt),
        scratch_shapes=[
            pltpu.VMEM((_NB, sq, d), dt),
            pltpu.VMEM((_NB, sk, d), dt),
            pltpu.VMEM((_NB, sk, d), dt),
            pltpu.VMEM((_NOS, _OG, sq, d), dt),
            pltpu.VMEM((sq, d), dt),
            pltpu.VMEM((sk, d), dt),
            pltpu.VMEM((sk, d), dt),
            pltpu.VMEM((sq, d), dt),
            pltpu.VMEM((sq, sk), jnp.float32),
            pltpu.VMEM((sq, _LANES), jnp.float32),
            pltpu.SemaphoreType.DMA((_NB,)),
            pltpu.SemaphoreType.DMA((_NB,)),
            pltpu.SemaphoreType.DMA((_NB,)),
            pltpu.SemaphoreType.DMA((_NOS,)),
            pltpu.SemaphoreType.DMA((2,)),
            pltpu.SemaphoreType.DMA((2,)),
        ],
        compiler_params=pltpu.CompilerParams(
            vmem_limit_bytes=100 * 1024 * 1024,
            flags={"XLA_TPU_RESCHEDULE_DMA_DONES": True},
            disable_bounds_checks=True,
        ),
    )(q.reshape(bh, sq, d), k.reshape(bh, sk, d), v.reshape(bh, sk, d))
    return out.reshape(b, h, sq, d)
```

```python
import jax
import jax.numpy as jnp
import numpy as np
from jax import lax
import jax.experimental.pallas as pl
import jax.experimental.pallas.tpu as pltpu

_LOG2E = 1.4426950408889634
_NT = (((1,), (1,)), ((), ()))
_NN = (((1,), (0,)), ((), ()))

_LANES = 128
_CK = 512
_U = 21
_T = 3
_NB = 7
_OG = 7
_NOS = 2 * (_U // _OG)


def _stage(q_ref, k_ref, v_ref, o_ref, s_in, m_in, r_prev, inv_prev, true_mask, scale,
           pv_first=False):
    do_qk = q_ref is not None
    do_pv = v_ref is not None
    pace = true_mask is not None
    sk = (k_ref if do_qk else v_ref).shape[0]
    nt = _CK // _LANES
    s_out = []
    m_run = l_run = acc = qh = None
    if do_qk:
        qs = q_ref[...].astype(jnp.float32) * scale
        if not pv_first:
            qh = qs.astype(jnp.bfloat16)

    def qk_chunk(j):
        nonlocal m_run
        keys = pl.ds(j * _CK, _CK)
        s = lax.dot_general(qh, k_ref[keys, :], _NT, preferred_element_type=jnp.float32)
        tiles = [s[:, t * _LANES:(t + 1) * _LANES] for t in range(nt)]
        s_out.append((s, tiles))
        mx = jnp.maximum(jnp.maximum(tiles[0], tiles[1]), jnp.maximum(tiles[2], tiles[3]))
        m_run = mx if m_run is None else jnp.maximum(m_run, mx)

    def pv_chunk(j):
        nonlocal l_run, acc, r_prev
        keys = pl.ds(j * _CK, _CK)
        m_j = m_in
        if pace and r_prev is not None:
            m_j = jnp.where(true_mask, m_in, r_prev)
        if pace and inv_prev is not None and j == 0:
            r = m_j.shape[0] - 16
            tok = [inv_prev[i:i + 8] for i in range(0, inv_prev.shape[0], 8)]
            while len(tok) > 1:
                tok = [jnp.maximum(*tok[i:i + 2]) if i + 1 < len(tok) else tok[i]
                       for i in range(0, len(tok), 2)]
            mid = jnp.where(true_mask[0:8], m_j[r:r + 8], tok[0])
            m_j = jnp.concatenate([m_j[:r], mid, m_j[r + 8:]], axis=0)
        p = [jnp.exp2(s_in(j, t) - m_j) for t in range(nt)]
        part = (p[0] + p[1]) + (p[2] + p[3])
        l_run = part if l_run is None else l_run + part
        if pace:
            for t in (1, 3):
                p[t] = jnp.minimum(p[t], l_run)
        pb = jnp.concatenate(p, axis=1).astype(jnp.bfloat16)
        r_prev = lax.dot_general(pb, v_ref[keys, :], _NN, preferred_element_type=jnp.float32)
        acc = r_prev if acc is None else acc + r_prev
        return p

    for j in range(sk // _CK):
        if pv_first and j == 0:
            p = pv_chunk(j)
            head = jnp.where(true_mask[0:8], qs[0:8], p[nt - 1][0:8])
            qh = jnp.concatenate([head, qs[8:]], axis=0).astype(jnp.bfloat16)
            qk_chunk(j)
        else:
            if do_qk:
                qk_chunk(j)
            if do_pv:
                pv_chunk(j)

    m_out = inv = None
    if do_qk:
        m_out = jnp.broadcast_to(jnp.max(m_run, axis=-1, keepdims=True), m_run.shape)
    if do_pv:
        l = jnp.sum(l_run, axis=-1, keepdims=True)
        r0 = pltpu.reciprocal(l, approx=True)
        inv = r0 * (2.0 - l * r0)
        o_ref[...] = (acc * inv).astype(o_ref.dtype)
        inv = jnp.broadcast_to(inv, acc.shape)
    return s_out, m_out, r_prev, inv


def _make_kernel(bh, sq, sk, d):
    n_it = (bh - 1 - _T) // _U
    n_og = _U // _OG
    n_grp = n_it * n_og
    scale = np.float32(d ** -0.5 * _LOG2E)

    def kernel(q_hbm, k_hbm, v_hbm, o_hbm,
               ring, ob, q0b, k0b, vlb, otb, olb, s_buf, m_buf,
               isem, osem, psem, lsem):
        def in_copies(s, slot):
            sem = isem.at[slot]
            return [pltpu.make_async_copy(k_hbm.at[s + 1], ring.at[slot, pl.ds(0, sk)], sem),
                    pltpu.make_async_copy(q_hbm.at[s + 1], ring.at[slot, pl.ds(2 * sk, sq)], sem),
                    pltpu.make_async_copy(v_hbm.at[s], ring.at[slot, pl.ds(sk, sk)], sem)]

        def start_in(s, slot):
            for cp in in_copies(s, slot):
                cp.start()

        def wait_in(slot):
            pltpu.make_async_copy(ring.at[slot], ring.at[slot], isem.at[slot]).wait()

        def o_copy(n, slot):
            return pltpu.make_async_copy(
                ob.at[slot], o_hbm.at[pl.ds(n * _OG, _OG)], osem.at[slot])

        def store_scores(s_out, m_out):
            for j, (s, _) in enumerate(s_out):
                s_buf[:, pl.ds(j * _CK, _CK)] = s
            m_buf[...] = m_out

        def load_scores(j, t):
            return s_buf[:, pl.ds(j * _CK + t * _LANES, _LANES)]

        def make_true_mask():
            bits = lax.bitcast_convert_type(
                q0b[pl.ds(0, 8), :].astype(jnp.float32), jnp.int32)
            mask = (bits | 1) != 0
            return jnp.broadcast_to(mask.reshape(1, 8, _LANES),
                                    (sq // 8, 8, _LANES)).reshape(sq, _LANES)

        v_last = pltpu.make_async_copy(v_hbm.at[bh - 1], vlb, lsem.at[0])
        o_tail = pltpu.make_async_copy(otb, o_hbm.at[pl.ds(n_it * _U, _T)], lsem.at[1])
        o_last = pltpu.make_async_copy(olb, o_hbm.at[bh - 1], lsem.at[2])

        first = [pltpu.make_async_copy(q_hbm.at[0], q0b, psem.at[0]),
                 pltpu.make_async_copy(k_hbm.at[0], k0b, psem.at[1])]
        for cp in first:
            cp.start()

        def fill_slot(u, carry):
            for cp in in_copies(u, u):
                cp.start()
            return carry

        lax.fori_loop(0, _NB, fill_slot, 0)
        for cp in first:
            cp.wait()
        s_out, m_out, _, _ = _stage(
            q0b, k0b, None, None, None, None, None, None, None, scale)
        store_scores(s_out, m_out)

        def body(g, carry):
            true_mask = make_true_mask()
            s_in, m_in, r_prev, inv_prev = load_scores, m_buf[...], None, None
            for u in range(_U):
                n = g * n_og + u // _OG
                oslot = lax.rem(n, _NOS)
                if u % _OG == 0:
                    @pl.when(n >= _NOS)
                    def _():
                        o_copy(n - _NOS, oslot).wait()

                    @pl.when(n >= 1)
                    def _():
                        o_copy(n - 1, lax.rem(n + _NOS - 1, _NOS)).start()

                slot = u % _NB
                wait_in(slot)
                s_out, m_out, r_prev, inv_prev = _stage(
                    ring.at[slot, pl.ds(2 * sk, sq)], ring.at[slot, pl.ds(0, sk)],
                    ring.at[slot, pl.ds(sk, sk)], ob.at[oslot, u % _OG],
                    s_in, m_in, r_prev, inv_prev, true_mask, scale, pv_first=(u == 0))
                if u == _U - 1:
                    store_scores(s_out, m_out)
                else:
                    s_in = lambda j, t, s_out=s_out: s_out[j][1][t]
                    m_in = m_out

                s_next = g * _U + u + _NB
                if u + _NB - _U < _T:
                    start_in(s_next, slot)
                else:
                    @pl.when(g + 1 < n_it)
                    def _():
                        start_in(s_next, slot)

                if u + _NB == _U:
                    @pl.when(g + 1 == n_it)
                    def _():
                        v_last.start()
            return carry

        lax.fori_loop(0, n_it, body, 0)

        o_copy(n_grp - 1, (n_grp - 1) % _NOS).start()
        v_last.wait()
        true_mask = make_true_mask()
        s_in, m_in, r_prev, inv_prev = load_scores, m_buf[...], None, None
        for t in range(_T):
            wait_in(t)
            s_out, m_out, r_prev, inv_prev = _stage(
                ring.at[t, pl.ds(2 * sk, sq)], ring.at[t, pl.ds(0, sk)],
                ring.at[t, pl.ds(sk, sk)], otb.at[t],
                s_in, m_in, r_prev, inv_prev, true_mask, scale, pv_first=(t == 0))
            s_in = lambda j, t_, s_out=s_out: s_out[j][1][t_]
            m_in = m_out
        o_tail.start()
        _stage(None, None, vlb, olb, s_in, m_in, r_prev, inv_prev, true_mask, scale)
        o_last.start()
        for n in range(max(n_grp - _NOS, 0), n_grp):
            o_copy(n, n % _NOS).wait()
        o_tail.wait()
        o_last.wait()

    return kernel


@jax.jit
def pallas_standalone__mha_softmax__near_ridge_kernel(
    q: jax.Array,
    k: jax.Array,
    v: jax.Array,
):
    b, h, sq, d = q.shape
    sk = k.shape[2]
    bh = b * h
    assert d == _LANES and sk % _CK == 0 and sq % 16 == 0
    assert bh > _U + _T and (bh - 1 - _T) % _U == 0
    assert _U % _NB == 0 and _U % _OG == 0 and 0 < _T <= _NB

    dt = q.dtype
    out = pl.pallas_call(
        _make_kernel(bh, sq, sk, d),
        in_specs=[pl.BlockSpec(memory_space=pl.ANY)] * 3,
        out_specs=pl.BlockSpec(memory_space=pl.ANY),
        out_shape=jax.ShapeDtypeStruct((bh, sq, d), dt),
        scratch_shapes=[
            pltpu.VMEM((_NB, 2 * sk + sq, d), dt),
            pltpu.VMEM((_NOS, _OG, sq, d), dt),
            pltpu.VMEM((sq, d), dt),
            pltpu.VMEM((sk, d), dt),
            pltpu.VMEM((sk, d), dt),
            pltpu.VMEM((_T, sq, d), dt),
            pltpu.VMEM((sq, d), dt),
            pltpu.VMEM((sq, sk), jnp.float32),
            pltpu.VMEM((sq, _LANES), jnp.float32),
            pltpu.SemaphoreType.DMA((_NB,)),
            pltpu.SemaphoreType.DMA((_NOS,)),
            pltpu.SemaphoreType.DMA((2,)),
            pltpu.SemaphoreType.DMA((3,)),
        ],
        compiler_params=pltpu.CompilerParams(
            vmem_limit_bytes=64 * 1024 * 1024,
            flags={"XLA_TPU_RESCHEDULE_DMA_DONES": True},
            disable_bounds_checks=True,
        ),
    )(q.reshape(bh, sq, d), k.reshape(bh, sk, d), v.reshape(bh, sk, d))
    return out.reshape(b, h, sq, d)
```
